```python
import jax
import jax.numpy as jnp

def _softmax(x, axis=-1):
    return jax.nn.softmax(x, axis=axis)
def _gelu(x):
    return jax.nn.gelu(x, approximate=True)
def _silu(x):
    return jax.nn.silu(x)
def _sigmoid(x):
    return jax.nn.sigmoid(x)
def _layernorm(x, axis=-1, eps=1e-5):
    m = jnp.mean(x, axis=axis, keepdims=True)
    v = jnp.var(x, axis=axis, keepdims=True)
    return (x - m) / jnp.sqrt(v + eps)
def _scatter_add(tgt, idx, src, axis=0):
    return tgt.at[idx].add(src)
def _segment_sum(src, seg, n):
    return jax.ops.segment_sum(src, seg, n)
class _Rng:
    def __init__(self, key):
        self._k = key
    def _next(self):
        self._k, sub = jax.random.split(self._k)
        return sub
    def normal(self, shape):
        return jax.random.normal(self._next(), shape, dtype=jnp.bfloat16)
    def randint(self, lo, hi, shape):
        return jax.random.randint(self._next(), shape, lo, hi, dtype=jnp.int32)
    def uniform(self, shape, lo=0.0, hi=1.0):
        return jax.random.uniform(self._next(), shape, jnp.bfloat16, lo, hi)
    def permutation(self, n):
        return jax.random.permutation(self._next(), n)


kernel_name = 'gated_mix__sliding_block_cached__mixer_s_mlp__decode'

def setup_inputs():
    _rng = _Rng(jax.random.key(int.from_bytes(__import__("os").urandom(4), "little")))
    _w = (lambda a: (lambda t: t.astype(jnp.bfloat16) if jnp.issubdtype(t.dtype, jnp.floating) else t)(jnp.asarray(a)))
    def _A_setup():
        B, Sq, D = 1, 1, 576
        Hq, Hkv, Sk, Dh = 32, 16, 65536, 128
        assert Hq % Hkv == 0, (Hq, Hkv)
        return {
            "x": _w((lambda *s: _rng.normal(s) * 0.05)(B, Sq, D)),
            "k_cache": _w((lambda *s: _rng.normal(s) * 0.05)(B, Hkv, Sk, Dh)),
            "v_cache": _w((lambda *s: _rng.normal(s) * 0.05)(B, Hkv, Sk, Dh)),
            "wq": _w((lambda *s: _rng.normal(s) * 0.05)(D, Hq * Dh) * (D ** -0.5)),
            "wo": _w((lambda *s: _rng.normal(s) * 0.05)(Hq * Dh, D) * ((Hq * Dh) ** -0.5)),
        }
    _A_in = _A_setup()

    def _B_setup():
        B, S, D, F = 1, 1, 576, 4608
        return {
            "x":  _w((lambda *s: _rng.normal(s) * 0.05)(B, S, D)),
            "w1": _w((lambda *s: _rng.normal(s) * 0.05)(D, D) * (D ** -0.5)),
            "w2": _w((lambda *s: _rng.normal(s) * 0.05)(D, D) * (D ** -0.5)),
            "w3": _w((lambda *s: _rng.normal(s) * 0.05)(D, F) * (D ** -0.5)),
            "w4": _w((lambda *s: _rng.normal(s) * 0.05)(F, D) * (F ** -0.5)),
        }
    _B_in = _B_setup()

    return {
        "A_x": _A_in["x"],
        "A_k_cache": _A_in["k_cache"],
        "A_v_cache": _A_in["v_cache"],
        "A_wq": _A_in["wq"],
        "A_wo": _A_in["wo"],
        "B_x": _B_in["x"],
        "B_w1": _B_in["w1"],
        "B_w2": _B_in["w2"],
        "B_w3": _B_in["w3"],
        "B_w4": _B_in["w4"],
        "gate_w": _w((lambda *s: _rng.normal(s) * 0.05)(576)),
    }

def reference(A_x, A_k_cache, A_v_cache, A_wq, A_wo, B_x, B_w1, B_w2, B_w3, B_w4, gate_w):
    def _A_ref(x, k_cache, v_cache, wq, wo):
        B, Sq, D = x.shape
        Hq, Dh = 32, 128
        Hkv, Sk = k_cache.shape[1], k_cache.shape[2]
        W = min(4096, max(256, Sk // 4))
        rep = Hq // Hkv
        q = (lambda x, *d: x.transpose(*d))((x @ wq).reshape(B, Sq, Hq, Dh), 0, 2, 1, 3)
        k = jnp.repeat(k_cache[:, :, Sk - W:, :], rep, axis=1)
        v = jnp.repeat(v_cache[:, :, Sk - W:, :], rep, axis=1)
        scores = jnp.einsum("bhqd,bhkd->bhqk", q, k) * (Dh ** -0.5)
        p = _softmax(scores, axis=-1)
        o = jnp.einsum("bhqk,bhkd->bhqd", p, v)
        return (lambda x, *d: x.transpose(*d))(o, 0, 2, 1, 3).reshape(B, Sq, Hq * Dh) @ wo

    def _B_ref(x, w1, w2, w3, w4):
        B, S, D = x.shape
        h = _gelu(_layernorm(x, axis=-1) @ w1)
        c = D // 4
        g0 = jnp.pad(h[:, :, 0*c:1*c], ((0, 0), (1, 0), (0, 0)))[:, :S, :]
        g1 = jnp.pad(h[:, :, 1*c:2*c], ((0, 0), (0, 1), (0, 0)))[:, 1:, :]
        g2 = jnp.pad(h[:, :, 2*c:3*c], ((0, 0), (2, 0), (0, 0)))[:, :S, :]
        g3 = jnp.pad(h[:, :, 3*c:   ], ((0, 0), (0, 2), (0, 0)))[:, 2:, :]
        hs = jnp.concatenate([g0, g1, g2, g3], axis=-1) @ w2
        x1 = x + hs
        h2 = _gelu(_layernorm(x1, axis=-1) @ w3) @ w4
        return x1 + h2

    x = A_x
    g = _sigmoid((x * gate_w).sum(-1, keepdims=True))
    a = _A_ref(x, A_k_cache, A_v_cache, A_wq, A_wo)
    b = _B_ref(x, B_w1, B_w2, B_w3, B_w4)
    return g * a + (1 - g) * b
```

```python
import functools
import math

import jax
import jax.numpy as jnp
from jax import lax
import jax.experimental.pallas as pl
import jax.experimental.pallas.tpu as pltpu

F32 = jnp.float32
BF16 = jnp.bfloat16
NT = (((1,), (1,)), ((), ()))


def _nn(a, b):
    return jnp.dot(a, b, preferred_element_type=F32)


def _nt(a, b):
    return lax.dot_general(a, b, NT, preferred_element_type=F32)


def make(kv_streams=4, w_streams=4, manual_out=True, debug=False):
    D, HQ, HKV, DH, SK, W, F = 576, 32, 16, 128, 65536, 4096, 4608
    S0 = SK - W
    PIECE = 128

    def order(n, ns):
        l = n // ns
        return [s * l + j for j in range(l) for s in range(ns)]

    def kernel(x_hbm, k_hbm, v_hbm, wq_hbm, wo_hbm, w3_hbm, w4_hbm, g_hbm, o_hbm,
               kb, vb, wqb, wob, w3b, w4b, xb, gb, ob, q_s, o_s, u_s, ya_s, yb_s,
               sem_kv, sem_w, sem_small):

        def kv_start(which, h):
            src, dst = ((k_hbm, kb), (v_hbm, vb))[which]
            slot = (h % 2) * 2 + which
            for i, j in enumerate(order(W // PIECE, kv_streams)):
                pltpu.make_async_copy(src.at[h, pl.ds(S0 + j * PIECE, PIECE), :],
                                      dst.at[h, pl.ds(j * PIECE, PIECE), :],
                                      sem_kv.at[slot]).start(priority=i % 2)

        def kv_wait(which, h):
            dst = (kb, vb)[which]
            slot = (h % 2) * 2 + which
            pltpu.make_async_copy(dst.at[h], dst.at[h], sem_kv.at[slot]).wait()

        def w_start(src, dst, r0, rows, sem):
            half = src.shape[1] // 2
            n = rows // 8 * 2
            for i, j in enumerate(order(n, w_streams)):
                r = pl.ds(pl.multiple_of(r0 + (j // 2) * 8, 8), 8)
                c = pl.ds((j % 2) * half, half)
                pltpu.make_async_copy(src.at[r, c], dst.at[r, c], sem).start(priority=i % 2)

        def w_wait(dst, r0, rows, sem):
            d = dst.at[pl.ds(r0, rows), :]
            pltpu.make_async_copy(d, d, sem).wait()

        def w_start_all(src, dst, sem):
            def body(c, carry):
                w_start(src, dst, c * 64, 64, sem)
            lax.fori_loop(0, D // 64, body, None)

        small = [pltpu.make_async_copy(s, d, sem_small.at[i])
                 for i, (s, d) in enumerate(((x_hbm, xb), (g_hbm, gb)))]
        for c in small:
            c.start()
        w_start_all(wq_hbm, wqb, sem_w.at[0])
        kv_start(0, 0)
        for c in small:
            c.wait()
        x = xb[0].astype(F32)
        x8 = jnp.broadcast_to(x, (8, D)).astype(BF16)
        kv_start(1, 0)
        w_wait(wqb, 0, D, sem_w.at[0])

        row = lax.broadcasted_iota(jnp.int32, (8, DH), 0)

        def head(h, carry):
            last = h == HKV - 1

            @pl.when(jnp.logical_not(last))
            def _():
                kv_start(0, h + 1)

            @pl.when(last)
            def _():
                w_start(w3_hbm, w3b, 0, 128, sem_w.at[1])

            c0 = pl.multiple_of(h * 2 * DH, 2 * DH)
            q2 = _nn(x8, wqb[:, pl.ds(c0, 2 * DH)])
            q = jnp.where(row == 0, q2[:, :DH], q2[:, DH:]).astype(BF16)
            kv_wait(0, h)
            s = _nt(q, kb[h]) * (DH ** -0.5)
            m = jnp.max(s, axis=-1, keepdims=True)
            p = jnp.exp(s - m)
            l = jnp.sum(p, axis=-1, keepdims=True)
            p = p.astype(BF16)

            @pl.when(jnp.logical_not(last))
            def _():
                kv_start(1, h + 1)

            @pl.when(last)
            def _():
                w_start(w3_hbm, w3b, 128, 128, sem_w.at[1])

            kv_wait(1, h)
            o = _nn(p, vb[h]) / l
            o0 = jnp.broadcast_to(o[0:1], (8, DH))
            o1 = jnp.broadcast_to(o[1:2], (8, DH))
            o_s[:, pl.ds(c0, 2 * DH)] = jnp.concatenate([o0, o1], axis=1).astype(BF16)
            return carry

        lax.fori_loop(0, HKV, head, None)

        bx = x
        mu = jnp.mean(bx, axis=-1, keepdims=True)
        var = jnp.mean(jnp.square(bx - mu), axis=-1, keepdims=True)
        ln = (bx - mu) / jnp.sqrt(var + 1e-5)
        ln8 = jnp.broadcast_to(ln, (8, D)).astype(BF16)
        gw = gb[...].reshape(1, D).astype(F32)
        gate = jax.nn.sigmoid(jnp.sum(x * gw, axis=-1, keepdims=True))

        w_start(w3_hbm, w3b, 256, 128, sem_w.at[1])
        w_start(w3_hbm, w3b, 384, 192, sem_w.at[1])
        w_start(w4_hbm, w4b, 0, 128, sem_w.at[2])
        w_start(w4_hbm, w4b, 128, 128, sem_w.at[3])
        w_wait(w3b, 0, D, sem_w.at[1])

        def up(j, carry):
            r0 = 256 + j * 32
            w_start(w4_hbm, w4b, r0, 32, sem_w.at[4 + jnp.minimum(j // 4, 2)])
            c0 = pl.multiple_of(j * 512, 512)
            z = _nn(ln8, w3b[:, pl.ds(c0, 512)])
            u_s[:, pl.ds(c0, 512)] = jax.nn.gelu(z, approximate=True).astype(BF16)
            return carry

        lax.fori_loop(0, 9, up, None)
        w_start(w4_hbm, w4b, 544, 32, sem_w.at[6])

        def down(j, carry):
            r0 = pl.multiple_of(j * 128, 128)
            w_start(wo_hbm, wob, r0, 128, sem_w.at[7 + j])
            w_wait(w4b, r0, 128, sem_w.at[2 + j])
            yb_s[:, pl.ds(r0, 128)] = _nt(u_s[...], w4b[pl.ds(r0, 128), :])
            return carry

        lax.fori_loop(0, 4, down, None)
        w_start(wo_hbm, wob, 512, 64, sem_w.at[11])
        w_wait(w4b, 512, 64, sem_w.at[6])
        yb_s[:, 512:D] = _nt(u_s[...], w4b[512:D, :])

        def proj(j, carry):
            r0 = pl.multiple_of(j * 128, 128)
            w_wait(wob, r0, 128, sem_w.at[7 + j])
            ya_s[:, pl.ds(r0, 128)] = _nt(o_s[...], wob[pl.ds(r0, 128), :])
            return carry

        lax.fori_loop(0, 4, proj, None)
        w_wait(wob, 512, 64, sem_w.at[11])
        ya_s[:, 512:D] = _nt(o_s[...], wob[512:D, :])

        a = ya_s[0:1, :]
        b = bx + yb_s[0:1, :]
        if debug == "a":
            res = a
        elif debug == "h2":
            res = yb_s[0:1, :]
        elif debug == "g":
            res = jnp.broadcast_to(gate, (1, D))
        else:
            res = gate * a + (1.0 - gate) * b
        if manual_out:
            ob[0] = res.astype(BF16)
            c = pltpu.make_async_copy(ob, o_hbm, sem_small.at[0])
            c.start()
            c.wait()
        else:
            o_hbm[0] = res.astype(BF16)

    def f(A_x, A_k_cache, A_v_cache, A_wq, A_wo, B_x, B_w1, B_w2, B_w3, B_w4, gate_w):
        hbm = pl.BlockSpec(memory_space=pl.ANY)
        return pl.pallas_call(
            kernel,
            out_shape=jax.ShapeDtypeStruct((1, 1, D), BF16),
            in_specs=[hbm] * 8,
            out_specs=hbm if manual_out else pl.BlockSpec(memory_space=pltpu.VMEM),
            scratch_shapes=[
                pltpu.VMEM((HKV, W, DH), BF16), pltpu.VMEM((HKV, W, DH), BF16),
                pltpu.VMEM((D, HQ * DH), BF16), pltpu.VMEM((D, HQ * DH), BF16),
                pltpu.VMEM((D, F), BF16), pltpu.VMEM((D, F), BF16),
                pltpu.VMEM((1, 1, D), BF16), pltpu.VMEM((D,), BF16),
                pltpu.VMEM((1, 1, D), BF16),
                pltpu.VMEM((HKV, 8, DH), F32), pltpu.VMEM((8, HQ * DH), BF16), pltpu.VMEM((8, F), BF16),
                pltpu.VMEM((8, D), F32), pltpu.VMEM((8, D), F32),
                pltpu.SemaphoreType.DMA((4,)), pltpu.SemaphoreType.DMA((12,)), pltpu.SemaphoreType.DMA((3,)),
            ],
            compiler_params=pltpu.CompilerParams(
                vmem_limit_bytes=100 * 1024 * 1024,
                disable_bounds_checks=True, disable_semaphore_checks=True),
        )(A_x, A_k_cache.reshape(HKV, SK, DH), A_v_cache.reshape(HKV, SK, DH), A_wq, A_wo.T,
          B_w3, B_w4.T, gate_w)

    return f


@jax.jit
def pallas_gated_mix__sliding_block_cached__mixer_s_mlp__decode_kernel(
    A_x, A_k_cache, A_v_cache, A_wq, A_wo, B_x, B_w1, B_w2, B_w3, B_w4, gate_w,
):
    return make(manual_out=False)(A_x, A_k_cache, A_v_cache, A_wq, A_wo, B_x, B_w1, B_w2, B_w3, B_w4, gate_w)
```

```python
import jax
import jax.numpy as jnp
from jax import lax
import jax.experimental.pallas as pl
import jax.experimental.pallas.tpu as pltpu

F32 = jnp.float32
BF16 = jnp.bfloat16
NT = (((1,), (1,)), ((), ()))


def _nn(a, b):
    return jnp.dot(a, b, preferred_element_type=F32)


def _nt(a, b):
    return lax.dot_general(a, b, NT, preferred_element_type=F32)


def make(manual_out=True, debug=False, nocomp=(), tail_cols=(2048, 2048), checks=False,
         v_split=8, pv_issue=10, wo_streams=2, prefill=2, end_skew=32, k_shift=0, v_shift=64):
    D, HQ, HKV, DH, SK, W, F = 576, 32, 16, 128, 65536, 4096, 4608
    S0 = SK - W
    A = HQ * DH
    NTAIL = len(tail_cols)
    tail_off = [sum(tail_cols[:i]) for i in range(NTAIL)]
    NB = W // 128

    def kernel(x_hbm, k_hbm, v_hbm, wq_hbm, wo_hbm, w3_hbm, w4_hbm, g_hbm, o_hbm,
               kb, vb, wqb, wob, w3b, w4b, xb, gb, ob, q_s, p_s, l_s, o_s, u_s, ya_s, yb_s, sems):
        (S_X, S_G, S_WQ, S_K, S_VA, S_VB, S_W3, S_W4, S_WO) = range(9)
        S_TAIL = S_WO + 4

        def mult(r, m):
            return r if isinstance(r, int) else pl.multiple_of(r, m)

        def kv_copy(src, dst, sem, h, r, rows, p):
            pltpu.make_async_copy(src.at[h, pl.ds(S0 + r, rows), :], dst.at[h, pl.ds(r, rows), :],
                                  sems.at[sem]).start(priority=p)

        def kv_step(src, dst, sem, h0, nh, t, shift):
            parts = HKV // nh
            nt = NB // parts

            def whole():
                for s in range(parts):
                    for h in range(nh // 2):
                        for p in range(2):
                            kv_copy(src, dst, sem, h0 + h + p * (nh // 2),
                                    mult((s * nt + t) * 128 + shift, 64), 128, p)

            def wrapped():
                for s in range(parts - 1):
                    for h in range(nh // 2):
                        for p in range(2):
                            kv_copy(src, dst, sem, h0 + h + p * (nh // 2), (s + 1) * nt * 128 - 128 + shift, 128, p)
                for r, rows in ((W - 128 + shift, 128 - shift), (0, shift)):
                    for h in range(nh // 2):
                        for p in range(2):
                            kv_copy(src, dst, sem, h0 + h + p * (nh // 2), r, rows, p)

            if shift == 0:
                whole()
            elif isinstance(t, int):
                wrapped() if t == nt - 1 else whole()
            else:
                pl.when(t < nt - 1)(whole)
                pl.when(t == nt - 1)(wrapped)

        def w_copy(src, dst, sem, r, c, cols, p):
            idx = (pl.ds(mult(r, 8), 8), pl.ds(c, cols))
            pltpu.make_async_copy(src.at[idx], dst.at[idx], sems.at[sem]).start(priority=p)

        def w_step(src, dst, sem, t, cols, prio=None):
            for c in range(0, src.shape[1], cols):
                for s in range(8):
                    w_copy(src, dst, sem, s * 72 + t * 8, c, cols, s % 2 if prio is None else prio)

        def steps(fn, lo, hi):
            lax.fori_loop(lo, hi, lambda i, c: fn(i), None)

        def wait(dst, sem):
            pltpu.make_async_copy(dst, dst, sems.at[sem]).wait()

        wq_step = lambda t, prio=None: w_step(wq_hbm, wqb, S_WQ, t, 2048, prio)
        w3_step = lambda t: w_step(w3_hbm, w3b, S_W3, t, 1536)
        w4_step = lambda t: w_step(w4_hbm, w4b, S_W4, t, 1536)
        k_step = lambda t: kv_step(k_hbm, kb, S_K, 0, HKV, t, k_shift)
        va_step = lambda t: kv_step(v_hbm, vb, S_VA, 0, v_split, t, v_shift)
        vb_step = lambda t: kv_step(v_hbm, vb, S_VB, v_split, HKV - v_split, t, v_shift)
        NA = NB * v_split // HKV

        wo_list = []
        for j in range(4):
            per = 16 // wo_streams
            for t in range(per):
                for c in (0, 2048):
                    for s in range(wo_streams):
                        wo_list.append((j * 128 + (s * per + t) * 8, c, 2048, S_WO + j))
        for i in range(NTAIL):
            for c in range(tail_off[i], tail_off[i] + tail_cols[i], 2048):
                cc = min(2048, tail_off[i] + tail_cols[i] - c)
                for t in range(4):
                    for s in range(2):
                        wo_list.append((512 + (s * 4 + t) * 8, c, cc, S_TAIL + i))

        if end_skew:
            early, late = wo_list[-2 * end_skew:-end_skew], wo_list[-end_skew:]
            wo_list = wo_list[:-2 * end_skew] + [e for pair in zip(early, late) for e in pair]

        def wo_issue(lo, hi):
            for i in range(lo, min(hi, len(wo_list))):
                r, c, cc, sem = wo_list[i]
                w_copy(wo_hbm, wob, sem, r, c, cc, i % 2)

        for t in range(prefill):
            wq_step(t, 1)
        x_copy = pltpu.make_async_copy(x_hbm, xb, sems.at[S_X])
        g_copy = pltpu.make_async_copy(g_hbm, gb, sems.at[S_G])
        x_copy.start()
        g_copy.start()
        steps(wq_step, prefill, 9)
        steps(w3_step, 0, 3)

        x_copy.wait()
        g_copy.wait()
        x = xb[0].astype(F32)
        x8 = jnp.broadcast_to(x, (8, D)).astype(BF16)
        mu = jnp.mean(x, axis=-1, keepdims=True)
        var = jnp.mean(jnp.square(x - mu), axis=-1, keepdims=True)
        ln8 = jnp.broadcast_to((x - mu) / jnp.sqrt(var + 1e-5), (8, D)).astype(BF16)
        gw = gb[...].reshape(1, D).astype(F32)
        gate = jax.nn.sigmoid(jnp.sum(x * gw, axis=-1, keepdims=True))
        row = lax.broadcasted_iota(jnp.int32, (8, DH), 0)

        wait(wqb, S_WQ)

        def q_body(i):
            @pl.when(i < 6)
            def _():
                w3_step(3 + i)

            @pl.when(i >= 6)
            def _():
                w4_step(i - 6)

            if "attn" in nocomp:
                return
            c0 = pl.multiple_of(i * 4 * DH, 4 * DH)
            q4 = _nn(x8, wqb[:, pl.ds(c0, 4 * DH)])
            for j in range(2):
                q_s[2 * i + j] = jnp.where(row == 0, q4[:, 2 * j * DH:(2 * j + 1) * DH],
                                           q4[:, (2 * j + 1) * DH:(2 * j + 2) * DH])

        steps(q_body, 0, 8)
        w4_step(2)
        wait(w3b, S_W3)

        def up_body(j):
            @pl.when(j < 6)
            def _():
                w4_step(3 + j)

            @pl.when(j >= 6)
            def _():
                k_step(j - 6)

            if "mlp" in nocomp:
                return
            c0 = pl.multiple_of(j * 512, 512)
            z = _nn(ln8, w3b[:, pl.ds(c0, 512)])
            u_s[:, pl.ds(c0, 512)] = jax.nn.gelu(z, approximate=True).astype(BF16)

        steps(up_body, 0, 9)
        k_step(3)
        wait(w4b, S_W4)

        def down_body(j):
            k_step(4 + j)
            if "mlp" in nocomp:
                return
            r0 = pl.multiple_of(j * 128, 128)
            yb_s[:, pl.ds(r0, 128)] = _nt(u_s[...], w4b[pl.ds(r0, 128), :])

        steps(down_body, 0, 4)
        if "mlp" not in nocomp:
            yb_s[:, 512:D] = _nt(u_s[...], w4b[512:D, :])
        b = x + yb_s[0:1, :]
        steps(k_step, 8, NB)
        steps(va_step, 0, 4)
        wait(kb, S_K)

        def scores(h):
            if "attn" in nocomp:
                return
            s = _nt(q_s[h].astype(BF16), kb[h]) * (DH ** -0.5)
            m = jnp.max(s, axis=-1, keepdims=True)
            p = jnp.exp(s - m)
            l_s[h] = jnp.broadcast_to(jnp.sum(p, axis=-1, keepdims=True), (8, DH))
            p_s[h] = p.astype(BF16)

        def pv(h):
            if "attn" in nocomp:
                return
            o = _nn(p_s[h], vb[h]) / l_s[h]
            c0 = mult(h * 2 * DH, 2 * DH)
            o2 = jnp.concatenate([jnp.broadcast_to(o[0:1], (8, DH)), jnp.broadcast_to(o[1:2], (8, DH))], axis=1)
            o_s[:, pl.ds(c0, 2 * DH)] = o2.astype(BF16)

        def v_step(t):
            @pl.when(t < NA)
            def _():
                va_step(t)

            @pl.when(t >= NA)
            def _():
                vb_step(t - NA)

        def score_body(h):
            v_step(4 + h)
            scores(h)

        steps(score_body, 0, HKV)
        first = max(20, NA + 4)
        steps(v_step, 20, first)
        wait(vb.at[pl.ds(0, v_split)], S_VA)

        def pva_body(i):
            @pl.when(first + i < NB)
            def _():
                v_step(first + i)

            pv(2 * i)
            pv(2 * i + 1)

        steps(pva_body, 0, v_split // 2)
        steps(v_step, min(NB, first + v_split // 2), NB)
        wo_issue(0, 64)
        wait(vb.at[pl.ds(v_split, HKV - v_split)], S_VB)
        n = 64
        for h in range(v_split, HKV, 2):
            pv(h)
            pv(h + 1)
            wo_issue(n, n + pv_issue)
            n += pv_issue

        for j in range(4):
            upto = len(wo_list) if j >= 1 else n
            wo_issue(n, upto)
            n = max(n, upto)
            wait(wob.at[pl.ds(j * 128, 128), :], S_WO + j)
            if "proj" not in nocomp:
                ya_s[:, j * 128:(j + 1) * 128] = _nt(o_s[...], wob[j * 128:(j + 1) * 128, :])

        acc = jnp.zeros((8, 64), F32)
        for i in range(NTAIL):
            cs = pl.ds(tail_off[i], tail_cols[i])
            wait(wob.at[pl.ds(512, 64), cs], S_TAIL + i)
            if "last" not in nocomp:
                acc = acc + _nt(o_s[:, cs], wob[pl.ds(512, 64), cs])
        ya_s[:, 512:D] = acc

        a = ya_s[0:1, :]
        if debug == "a":
            res = a
        elif debug == "h2":
            res = yb_s[0:1, :]
        elif debug == "g":
            res = jnp.broadcast_to(gate, (1, D))
        else:
            res = gate * a + (1.0 - gate) * b
        if manual_out:
            ob[0] = res.astype(BF16)
            c = pltpu.make_async_copy(ob, o_hbm, sems.at[S_X])
            c.start()
            c.wait()
        else:
            o_hbm[0] = res.astype(BF16)

    def f(A_x, A_k_cache, A_v_cache, A_wq, A_wo, B_x, B_w1, B_w2, B_w3, B_w4, gate_w):
        hbm = pl.BlockSpec(memory_space=pl.ANY)
        return pl.pallas_call(
            kernel,
            out_shape=jax.ShapeDtypeStruct((1, 1, D), BF16),
            in_specs=[hbm] * 8,
            out_specs=hbm if manual_out else pl.BlockSpec(memory_space=pltpu.VMEM),
            scratch_shapes=[
                pltpu.VMEM((HKV, W, DH), BF16), pltpu.VMEM((HKV, W, DH), BF16),
                pltpu.VMEM((D, A), BF16), pltpu.VMEM((D, A), BF16),
                pltpu.VMEM((D, F), BF16), pltpu.VMEM((D, F), BF16),
                pltpu.VMEM((1, 1, D), BF16), pltpu.VMEM((D,), BF16), pltpu.VMEM((1, 1, D), BF16),
                pltpu.VMEM((HKV, 8, DH), F32), pltpu.VMEM((HKV, 8, W), BF16), pltpu.VMEM((HKV, 8, DH), F32),
                pltpu.VMEM((8, A), BF16), pltpu.VMEM((8, F), BF16),
                pltpu.VMEM((8, D), F32), pltpu.VMEM((8, D), F32),
                pltpu.SemaphoreType.DMA((12 + NTAIL,)),
            ],
            compiler_params=pltpu.CompilerParams(
                vmem_limit_bytes=100 * 1024 * 1024,
                disable_bounds_checks=not checks, disable_semaphore_checks=not checks),
        )(A_x, A_k_cache.reshape(HKV, SK, DH), A_v_cache.reshape(HKV, SK, DH), A_wq, A_wo.T,
          B_w3, B_w4.T, gate_w)

    return f


@jax.jit
def pallas_gated_mix__sliding_block_cached__mixer_s_mlp__decode_kernel(
    A_x, A_k_cache, A_v_cache, A_wq, A_wo, B_x, B_w1, B_w2, B_w3, B_w4, gate_w,
):
    return make(v_shift=64)(A_x, A_k_cache, A_v_cache, A_wq, A_wo, B_x, B_w1, B_w2, B_w3, B_w4, gate_w)
```

```python
import jax
import jax.numpy as jnp
from jax import lax
import jax.experimental.pallas as pl
import jax.experimental.pallas.tpu as pltpu

F32 = jnp.float32
BF16 = jnp.bfloat16

D, FF = 576, 4608
HQ, HKV, DH = 32, 16, 128
SK, WINDOW = 65536, 4096
ATTN = HQ * DH
FIRST_ROW = SK - WINDOW
LN_EPS = 1e-5

KV_ROWS = 128
V_CUT = 64
V_GROUP = HKV // 2
HEAD_START = 28
WO_TILE = 128
WO_FULL = D // WO_TILE
WO_REST = WO_FULL * WO_TILE
WO_LAST_COLS = ATTN // 2

SEM_X, SEM_GATE, SEM_WQ, SEM_W3, SEM_W4, SEM_K, SEM_V = range(7)
SEM_WO = SEM_V + 2
SEM_WO_REST = SEM_WO + WO_FULL
NUM_SEMS = SEM_WO_REST + ATTN // WO_LAST_COLS


def _nn(a, b):
    return jnp.dot(a, b, preferred_element_type=F32)


def _nt(a, b):
    return lax.dot_general(a, b, (((1,), (1,)), ((), ())), preferred_element_type=F32)


def _aligned(i, n):
    return i if isinstance(i, int) else pl.multiple_of(i, n)


def _loop(lo, hi, body):
    lax.fori_loop(lo, hi, lambda i, carry: body(i), None)


def _wq_plan():
    pieces = [(64 * s + 8 * t, c)
              for t in range(8) for c in (0, 2048) for s in (0, 5, 1, 6, 2, 7, 3, 8, 4)]
    return [(r, c, 1 if i < HEAD_START else (i - HEAD_START) % 2) for i, (r, c) in enumerate(pieces)]


def _wo_plan():
    pieces = [(WO_TILE * j + 32 * s + 8 * t, c, SEM_WO + j)
              for j in range(WO_FULL) for t in range(4) for c in (0, 2048) for s in range(4)]
    pieces += [(WO_REST + 32 * s + 8 * t, WO_LAST_COLS * j, SEM_WO_REST + j)
               for j in range(ATTN // WO_LAST_COLS) for t in range(4) for s in range(2)]
    early, late = pieces[-64:-32], pieces[-32:]
    pieces = pieces[:-64] + [p for pair in zip(early, late) for p in pair]
    return [piece + (i % 2,) for i, piece in enumerate(pieces)]


def _kernel(x_hbm, gate_hbm, k_hbm, v_hbm, wq_hbm, wo_hbm, w3_hbm, w4_hbm, out_ref,
            x_buf, gate_buf, k_buf, v_buf, wq_buf, wo_buf, w3_buf, w4_buf,
            q_ref, p_ref, psum_ref, o_ref, u_ref, attn_ref, mlp_ref, sems):

    def start_kv(src, dst, sem, head, heads_per_queue, row, rows):
        for h in range(heads_per_queue):
            for prio in range(2):
                hh = head + h + prio * heads_per_queue
                pltpu.make_async_copy(src.at[hh, pl.ds(FIRST_ROW + row, rows), :],
                                      dst.at[hh, pl.ds(row, rows), :],
                                      sems.at[sem]).start(priority=prio)

    def start_weight(src, dst, sem, row, col, cols, prio):
        piece = (pl.ds(_aligned(row, 8), 8), pl.ds(col, cols))
        pltpu.make_async_copy(src.at[piece], dst.at[piece], sems.at[sem]).start(priority=prio)

    def wait(filled, sem):
        pltpu.make_async_copy(filled, filled, sems.at[sem]).wait()

    def mlp_weight_step(src, dst, sem, t):
        for c in range(0, FF, FF // 3):
            for s in range(8):
                start_weight(src, dst, sem, D // 8 * s + 8 * t, c, FF // 3, s % 2)

    def w3_step(t):
        mlp_weight_step(w3_hbm, w3_buf, SEM_W3, t)

    def w4_step(t):
        mlp_weight_step(w4_hbm, w4_buf, SEM_W4, t)

    def k_step(t):
        start_kv(k_hbm, k_buf, SEM_K, 0, HKV // 2, _aligned(t * KV_ROWS, KV_ROWS), KV_ROWS)

    def v_step(t):
        group, u = t // 16, t % 16

        def start(row, rows):
            start_kv(v_hbm, v_buf, SEM_V + group, group * V_GROUP, V_GROUP // 2, row, rows)

        @pl.when(u < 15)
        def _():
            start(_aligned(V_CUT + u * KV_ROWS, V_CUT), KV_ROWS)
            start(_aligned(V_CUT + (u + 16) * KV_ROWS, V_CUT), KV_ROWS)

        @pl.when(u == 15)
        def _():
            start(V_CUT + 15 * KV_ROWS, KV_ROWS)
            start(WINDOW - KV_ROWS + V_CUT, KV_ROWS - V_CUT)
            start(0, V_CUT)

    wo_plan = _wo_plan()

    def start_wo(lo, hi):
        for row, col, sem, prio in wo_plan[lo:hi]:
            start_weight(wo_hbm, wo_buf, sem, row, col, 2048, prio)

    x_copy = pltpu.make_async_copy(x_hbm, x_buf, sems.at[SEM_X])
    gate_copy = pltpu.make_async_copy(gate_hbm, gate_buf, sems.at[SEM_GATE])
    x_copy.start(priority=1)
    gate_copy.start(priority=1)
    for row, col, prio in _wq_plan():
        start_weight(wq_hbm, wq_buf, SEM_WQ, row, col, 2048, prio)
    _loop(0, 3, w3_step)

    x_copy.wait()
    gate_copy.wait()
    x = x_buf[0].astype(F32)
    gate = jax.nn.sigmoid(jnp.sum(x * gate_buf[...].reshape(1, D).astype(F32), axis=-1, keepdims=True))
    mean = jnp.mean(x, axis=-1, keepdims=True)
    var = jnp.mean(jnp.square(x - mean), axis=-1, keepdims=True)
    x_rows = jnp.broadcast_to(x, (8, D)).astype(BF16)
    ln_rows = jnp.broadcast_to((x - mean) / jnp.sqrt(var + LN_EPS), (8, D)).astype(BF16)

    wait(wq_buf, SEM_WQ)
    first_row = lax.broadcasted_iota(jnp.int32, (8, DH), 0) == 0

    def queries(i):
        pl.when(i < 6)(lambda: w3_step(3 + i))
        pl.when(i >= 6)(lambda: w4_step(i - 6))
        q = _nn(x_rows, wq_buf[:, pl.ds(_aligned(i * 4 * DH, 4 * DH), 4 * DH)])
        for j in range(2):
            q_ref[2 * i + j] = jnp.where(first_row, q[:, 2 * j * DH:(2 * j + 1) * DH],
                                         q[:, (2 * j + 1) * DH:(2 * j + 2) * DH])

    _loop(0, HKV // 2, queries)
    w4_step(2)

    wait(w3_buf, SEM_W3)

    def mlp_up(i):
        pl.when(i < 6)(lambda: w4_step(3 + i))
        pl.when(i >= 6)(lambda: k_step(i - 6))
        cols = pl.ds(_aligned(i * 512, 512), 512)
        u_ref[:, cols] = jax.nn.gelu(_nn(ln_rows, w3_buf[:, cols]), approximate=True).astype(BF16)

    _loop(0, FF // 512, mlp_up)
    k_step(3)
    wait(w4_buf, SEM_W4)

    def mlp_down(i):
        _loop(4 + 2 * i, 6 + 2 * i, k_step)
        rows = pl.ds(_aligned(i * 128, 128), 128)
        mlp_ref[:, rows] = _nt(u_ref[...], w4_buf[rows, :])

    _loop(0, 4, mlp_down)
    mlp_ref[:, 512:D] = _nt(u_ref[...], w4_buf[512:D, :])
    _loop(12, WINDOW // KV_ROWS, k_step)
    _loop(0, 4, v_step)

    wait(k_buf, SEM_K)

    def probabilities(h):
        v_step(4 + h)
        s = _nt(q_ref[h].astype(BF16), k_buf[h]) * DH ** -0.5
        p = jnp.exp(s - jnp.max(s, axis=-1, keepdims=True))
        psum_ref[h] = jnp.broadcast_to(jnp.sum(p, axis=-1, keepdims=True), (8, DH))
        p_ref[h] = p.astype(BF16)

    def weighted_values(h):
        o = _nn(p_ref[h], v_buf[h]) / psum_ref[h]
        heads = [jnp.broadcast_to(o[r:r + 1], (8, DH)) for r in range(2)]
        o_ref[:, pl.ds(_aligned(h * 2 * DH, 2 * DH), 2 * DH)] = jnp.concatenate(heads, axis=1).astype(BF16)

    _loop(0, HKV, probabilities)
    wait(v_buf.at[pl.ds(0, V_GROUP)], SEM_V)

    def first_group(i):
        v_step(4 + HKV + i)
        weighted_values(2 * i)
        weighted_values(2 * i + 1)

    _loop(0, V_GROUP // 2, first_group)
    _loop(4 + HKV + V_GROUP // 2, 32, v_step)
    start_wo(0, 64)
    wait(v_buf.at[pl.ds(V_GROUP, V_GROUP)], SEM_V + 1)

    def second_group(i):
        for j in range(V_GROUP // 2):
            pl.when(i == j)(lambda j=j: start_wo(64 + 20 * j, 84 + 20 * j))
        weighted_values(V_GROUP + 2 * i)
        weighted_values(V_GROUP + 2 * i + 1)

    _loop(0, V_GROUP // 2, second_group)

    for j in range(WO_FULL):
        rows = pl.ds(j * WO_TILE, WO_TILE)
        wait(wo_buf.at[rows, :], SEM_WO + j)
        attn_ref[:, rows] = _nt(o_ref[...], wo_buf[rows, :])

    rows = pl.ds(WO_REST, D - WO_REST)
    for j in range(ATTN // WO_LAST_COLS):
        cols = pl.ds(j * WO_LAST_COLS, WO_LAST_COLS)
        wait(wo_buf.at[rows, cols], SEM_WO_REST + j)
        part = _nt(o_ref[:, cols], wo_buf[rows, cols])
        attn_ref[:, rows] = part if j == 0 else attn_ref[:, rows] + part

    out_ref[0] = (gate * attn_ref[0:1, :] + (1.0 - gate) * (x + mlp_ref[0:1, :])).astype(out_ref.dtype)


@jax.jit
def pallas_gated_mix__sliding_block_cached__mixer_s_mlp__decode_kernel(
    A_x: jax.Array,
    A_k_cache: jax.Array,
    A_v_cache: jax.Array,
    A_wq: jax.Array,
    A_wo: jax.Array,
    B_x: jax.Array,
    B_w1: jax.Array,
    B_w2: jax.Array,
    B_w3: jax.Array,
    B_w4: jax.Array,
    gate_w: jax.Array,
):
    del B_x, B_w1, B_w2
    assert A_x.shape == (1, 1, D)
    assert A_k_cache.shape == A_v_cache.shape == (1, HKV, SK, DH)
    assert A_wq.shape == (D, ATTN) and A_wo.shape == (ATTN, D)
    assert B_w3.shape == (D, FF) and B_w4.shape == (FF, D)

    in_hbm = pl.BlockSpec(memory_space=pl.ANY)
    return pl.pallas_call(
        _kernel,
        out_shape=jax.ShapeDtypeStruct((1, 1, D), A_x.dtype),
        in_specs=[in_hbm] * 8,
        out_specs=pl.BlockSpec(memory_space=pltpu.VMEM),
        scratch_shapes=[
            pltpu.VMEM((1, 1, D), BF16),
            pltpu.VMEM((D,), BF16),
            pltpu.VMEM((HKV, WINDOW, DH), BF16),
            pltpu.VMEM((HKV, WINDOW, DH), BF16),
            pltpu.VMEM((D, ATTN), BF16),
            pltpu.VMEM((D, ATTN), BF16),
            pltpu.VMEM((D, FF), BF16),
            pltpu.VMEM((D, FF), BF16),
            pltpu.VMEM((HKV, 8, DH), F32),
            pltpu.VMEM((HKV, 8, WINDOW), BF16),
            pltpu.VMEM((HKV, 8, DH), F32),
            pltpu.VMEM((8, ATTN), BF16),
            pltpu.VMEM((8, FF), BF16),
            pltpu.VMEM((8, D), F32),
            pltpu.VMEM((8, D), F32),
            pltpu.SemaphoreType.DMA((NUM_SEMS,)),
        ],
        compiler_params=pltpu.CompilerParams(
            vmem_limit_bytes=64 * 1024 * 1024,
            disable_bounds_checks=True,
            disable_semaphore_checks=True,
        ),
    )(
        A_x, gate_w, A_k_cache.reshape(HKV, SK, DH), A_v_cache.reshape(HKV, SK, DH),
        A_wq, A_wo.T, B_w3, B_w4.T,
    )
```
